```python
import os as _os
_os.environ.setdefault("JAX_PLATFORMS", "cpu")
import jax
import jax.numpy as jnp

def _softmax(x, axis=-1):
    return jax.nn.softmax(x, axis=axis)
def _gelu(x):
    return jax.nn.gelu(x, approximate=True)
def _silu(x):
    return jax.nn.silu(x)
def _sigmoid(x):
    return jax.nn.sigmoid(x)
def _layernorm(x, axis=-1, eps=1e-5):
    m = jnp.mean(x, axis=axis, keepdims=True)
    v = jnp.var(x, axis=axis, keepdims=True)
    return (x - m) / jnp.sqrt(v + eps)
def _scatter_add(tgt, idx, src, axis=0):
    return tgt.at[idx].add(src)
def _segment_sum(src, seg, n):
    return jax.ops.segment_sum(src, seg, n)
class _Rng:
    def __init__(self, key):
        self._k = key
    def _next(self):
        self._k, sub = jax.random.split(self._k)
        return sub
    def normal(self, shape):
        return jax.random.normal(self._next(), shape, dtype=jnp.bfloat16)
    def randint(self, lo, hi, shape):
        return jax.random.randint(self._next(), shape, lo, hi, dtype=jnp.int32)
    def uniform(self, shape, lo=0.0, hi=1.0):
        return jax.random.uniform(self._next(), shape, jnp.bfloat16, lo, hi)
    def permutation(self, n):
        return jax.random.permutation(self._next(), n)


kernel_name = 'concat_heads__gqa_block_cached__mha_block_cached__near_ridge'

def setup_inputs():
    _rng = _Rng(jax.random.key(int.from_bytes(__import__("os").urandom(4), "little")))
    _w = (lambda a: (lambda t: t.astype(jnp.bfloat16) if jnp.issubdtype(t.dtype, jnp.floating) else t)(jnp.asarray(a)))
    def _A_setup():
        B, Sq, D = 16, 32, 512
        Hq, Hkv, Sk, Dh = 32, 8, 512, 128
        assert Hq % Hkv == 0, (Hq, Hkv)
        return {
            "x": _w((lambda *s: _rng.normal(s) * 0.8)(B, Sq, D)),
            "k_cache": _w((lambda *s: _rng.normal(s) * 0.8)(B, Hkv, Sk, Dh)),
            "v_cache": _w((lambda *s: _rng.normal(s) * 0.05)(B, Hkv, Sk, Dh)),
            "wq": _w((lambda *s: _rng.normal(s) * 0.8)(D, Hq * Dh) * (D ** -0.5)),
            "wo": _w((lambda *s: _rng.normal(s) * 0.05)(Hq * Dh, D) * ((Hq * Dh) ** -0.5)),
        }
    _A_in = _A_setup()

    def _B_setup():
        B, Sq, D = 16, 32, 512
        H, Sk, Dh = 32, 512, 128
        return {
            "x": _w((lambda *s: _rng.normal(s) * 0.8)(B, Sq, D)),
            "k_cache": _w((lambda *s: _rng.normal(s) * 0.8)(B, H, Sk, Dh)),
            "v_cache": _w((lambda *s: _rng.normal(s) * 0.05)(B, H, Sk, Dh)),
            "wq": _w((lambda *s: _rng.normal(s) * 0.8)(D, H * Dh) * (D ** -0.5)),
            "wo": _w((lambda *s: _rng.normal(s) * 0.05)(H * Dh, D) * ((H * Dh) ** -0.5)),
        }
    _B_in = _B_setup()

    return {
        "A_x": _A_in["x"],
        "A_k_cache": _A_in["k_cache"],
        "A_v_cache": _A_in["v_cache"],
        "A_wq": _A_in["wq"],
        "A_wo": _A_in["wo"],
        "B_x": _B_in["x"],
        "B_k_cache": _B_in["k_cache"],
        "B_v_cache": _B_in["v_cache"],
        "B_wq": _B_in["wq"],
        "B_wo": _B_in["wo"],
    }

def reference(A_x, A_k_cache, A_v_cache, A_wq, A_wo, B_x, B_k_cache, B_v_cache, B_wq, B_wo):
    def _A_ref(x, k_cache, v_cache, wq, wo):
        B, Sq, D = x.shape
        Hq, Dh = 32, 128
        Hkv = k_cache.shape[1]
        rep = Hq // Hkv
        q = (lambda x, *d: x.transpose(*d))((x @ wq).reshape(B, Sq, Hq, Dh), 0, 2, 1, 3)
        k = jnp.repeat(k_cache, rep, axis=1)
        v = jnp.repeat(v_cache, rep, axis=1)
        scores = jnp.einsum("bhqd,bhkd->bhqk", q, k) * (Dh ** -0.5)
        p = _softmax(scores, axis=-1)
        o = jnp.einsum("bhqk,bhkd->bhqd", p, v)
        return (lambda x, *d: x.transpose(*d))(o, 0, 2, 1, 3).reshape(B, Sq, Hq * Dh) @ wo

    def _B_ref(x, k_cache, v_cache, wq, wo):
        B, Sq, D = x.shape
        H, Dh = 32, 128
        q = (lambda x, *d: x.transpose(*d))((x @ wq).reshape(B, Sq, H, Dh), 0, 2, 1, 3)
        scores = jnp.einsum("bhqd,bhkd->bhqk", q, k_cache) * (Dh ** -0.5)
        p = _softmax(scores, axis=-1)
        o = jnp.einsum("bhqk,bhkd->bhqd", p, v_cache)
        return (lambda x, *d: x.transpose(*d))(o, 0, 2, 1, 3).reshape(B, Sq, H * Dh) @ wo

    a = _A_ref(A_x, A_k_cache, A_v_cache, A_wq, A_wo)
    b = _B_ref(B_x, B_k_cache, B_v_cache, B_wq, B_wo)
    return jnp.concatenate([a, b], axis=-1)
```

```python
import functools
import math

import jax
import jax.numpy as jnp
from jax import lax
import jax.experimental.pallas as pl
import jax.experimental.pallas.tpu as pltpu

_NT = (((1,), (1,)), ((), ()))
_LOG2E = math.log2(math.e)


def _attend(q, k, v):
    s = lax.dot_general(q, k, _NT, preferred_element_type=jnp.float32)
    m = jnp.max(s, axis=-1, keepdims=True)
    p = jnp.exp2(s - m)
    l = jnp.sum(p, axis=-1, keepdims=True)
    o = jnp.dot(p.astype(jnp.bfloat16), v, preferred_element_type=jnp.float32)
    return o * pl.reciprocal(l, approx=False)


def _kernel(xa_ref, ka_ref, va_ref, wqa_ref, woa_ref,
            xb_ref, kb_ref, vb_ref, wqb_ref, wob_ref,
            out_ref, acc_ref, *, bc, sq, dh, rep, d, qscale):
    g = pl.program_id(0)
    c = pl.program_id(1)
    rows = bc * sq
    r0 = pl.multiple_of(c * rows, rows)

    xa = xa_ref[pl.ds(r0, rows), :]
    qa = (jnp.dot(xa, wqa_ref[...], preferred_element_type=jnp.float32) * qscale).astype(jnp.bfloat16)
    oa_rows = []
    for b in range(bc):
        qb = jnp.concatenate(
            [qa[b * sq:(b + 1) * sq, r * dh:(r + 1) * dh] for r in range(rep)], axis=0)
        o = _attend(qb, ka_ref[b, 0], va_ref[b, 0]).astype(jnp.bfloat16)
        oa_rows.append(jnp.concatenate(
            [o[r * sq:(r + 1) * sq, :] for r in range(rep)], axis=1))
    oa = jnp.concatenate(oa_rows, axis=0)
    ya = jnp.dot(oa, woa_ref[...], preferred_element_type=jnp.float32)

    xb = xb_ref[pl.ds(r0, rows), :]
    qb_all = (jnp.dot(xb, wqb_ref[...], preferred_element_type=jnp.float32) * qscale).astype(jnp.bfloat16)
    ob_rows = []
    for b in range(bc):
        heads = []
        for r in range(rep):
            q = qb_all[b * sq:(b + 1) * sq, r * dh:(r + 1) * dh]
            heads.append(_attend(q, kb_ref[b, r], vb_ref[b, r]).astype(jnp.bfloat16))
        ob_rows.append(jnp.concatenate(heads, axis=1))
    ob = jnp.concatenate(ob_rows, axis=0)
    yb = jnp.dot(ob, wob_ref[...], preferred_element_type=jnp.float32)

    @pl.when(g == 0)
    def _():
        acc_ref[pl.ds(r0, rows), 0:d] = ya
        acc_ref[pl.ds(r0, rows), d:2 * d] = yb

    @pl.when(g > 0)
    def _():
        acc_ref[pl.ds(r0, rows), 0:d] += ya
        acc_ref[pl.ds(r0, rows), d:2 * d] += yb

    @pl.when(g == pl.num_programs(0) - 1)
    def _():
        out_ref[...] = acc_ref[pl.ds(r0, rows), :].astype(out_ref.dtype)


@jax.jit
def pallas_concat_heads__gqa_block_cached__mha_block_cached__near_ridge_kernel(
    A_x: jax.Array,
    A_k_cache: jax.Array,
    A_v_cache: jax.Array,
    A_wq: jax.Array,
    A_wo: jax.Array,
    B_x: jax.Array,
    B_k_cache: jax.Array,
    B_v_cache: jax.Array,
    B_wq: jax.Array,
    B_wo: jax.Array,
):
    B, Sq, D = A_x.shape
    _, Hkv, Sk, Dh = A_k_cache.shape
    H = B_k_cache.shape[1]
    rep = H // Hkv
    bc = 4
    nc = B // bc
    rows = bc * Sq
    gw = rep * Dh
    qscale = (Dh ** -0.5) * _LOG2E

    xa = A_x.reshape(B * Sq, D)
    xb = B_x.reshape(B * Sq, D)

    x_spec = pl.BlockSpec((B * Sq, D), lambda g, c: (0, 0))
    kva_spec = pl.BlockSpec((bc, 1, Sk, Dh), lambda g, c: (c, g, 0, 0))
    kvb_spec = pl.BlockSpec((bc, rep, Sk, Dh), lambda g, c: (c, g, 0, 0))
    wq_spec = pl.BlockSpec((D, gw), lambda g, c: (0, g))
    wo_spec = pl.BlockSpec((gw, D), lambda g, c: (g, 0))
    out_spec = pl.BlockSpec(
        (rows, 2 * D), lambda g, c: (jnp.where(g == Hkv - 1, c, 0), 0))

    out = pl.pallas_call(
        functools.partial(_kernel, bc=bc, sq=Sq, dh=Dh, rep=rep, d=D, qscale=qscale),
        grid=(Hkv, nc),
        in_specs=[x_spec, kva_spec, kva_spec, wq_spec, wo_spec,
                  x_spec, kvb_spec, kvb_spec, wq_spec, wo_spec],
        out_specs=out_spec,
        out_shape=jax.ShapeDtypeStruct((B * Sq, 2 * D), A_x.dtype),
        scratch_shapes=[pltpu.VMEM((B * Sq, 2 * D), jnp.float32)],
        compiler_params=pltpu.CompilerParams(
            dimension_semantics=("arbitrary", "arbitrary"),
            vmem_limit_bytes=64 * 1024 * 1024,
        ),
    )(xa, A_k_cache, A_v_cache, A_wq, A_wo, xb, B_k_cache, B_v_cache, B_wq, B_wo)
    return out.reshape(B, Sq, 2 * D)
```

```python
import functools
import math
import os

import jax
import jax.numpy as jnp
from jax import lax
import jax.experimental.pallas as pl
import jax.experimental.pallas.tpu as pltpu

_NT = (((1,), (1,)), ((), ()))
_LOG2E = math.log2(math.e)
NOCHK = int(os.environ.get('NOCHK', '1'))
KSPLIT = tuple(int(x) for x in os.environ.get('KSPLIT', '272,240').split(','))
VSPLIT = tuple(int(x) for x in os.environ.get('VSPLIT', '256,256').split(','))
NOCOMP = int(os.environ.get('NOCOMP', '0'))
NOW = int(os.environ.get('NOW', '0'))
ISSUE_FIRST = int(os.environ.get('ISSUE_FIRST', '0'))
NPAR = int(os.environ.get('NPAR', '2'))
LA = int(os.environ.get('LA', '7'))


def _scores(q, k):
    s = lax.dot_general(q, k, _NT, preferred_element_type=jnp.float32)
    m = jnp.max(s, axis=-1, keepdims=True)
    p = jnp.exp2(s - m)
    l = jnp.sum(p, axis=-1, keepdims=True)
    r = pl.reciprocal(l, approx=True)
    r = r * (2.0 - l * r)
    return p.astype(jnp.bfloat16), r


def _pv(p, r, v):
    o = jnp.dot(p, v, preferred_element_type=jnp.float32)
    return (o * r).astype(jnp.bfloat16)


def _kernel(xa_hbm, ka_hbm, va_hbm, wqa_hbm, woa_hbm,
            xb_hbm, kb_hbm, vb_hbm, wqb_hbm, wob_hbm,
            out_ref,
            acc_ref, x_buf, wq_buf, wo_buf,
            k0, k1, k2, k3, v0, v1, v2, v3,
            ksem, vsem, wqsem, wosem, xsem,
            *, nb, bc, sq, sk, dh, rep, d, hkv, qscale):
    g = pl.program_id(0)
    c = pl.program_id(1)
    rows = bc * sq
    gw = rep * dh
    r0 = pl.multiple_of(c * rows, rows)
    kbufs = (k0, k1, k2, k3)
    vbufs = (v0, v1, v2, v3)
    n_units = hkv * nb
    wrows = d // nb

    def issue_kv(gu, bu, slot, par):
        a_row = (bu * hkv + gu) * sk
        b_row = (bu * hkv + gu) * (rep * sk)
        for h in range(rep + 1):
            if h == 0:
                ks, vs, base = ka_hbm, va_hbm, a_row
            else:
                ks, vs, base = kb_hbm, vb_hbm, b_row + (h - 1) * sk
            ko = vo = 0
            for kn, vn in zip(KSPLIT, VSPLIT):
                pltpu.make_async_copy(
                    ks.at[pl.ds(pl.multiple_of(base + ko, 8), kn)],
                    kbufs[slot].at[par, pl.ds(h * sk + ko, kn)], ksem.at[par, slot]).start(priority=0)
                pltpu.make_async_copy(
                    vs.at[pl.ds(pl.multiple_of(base + vo, 8), vn)],
                    vbufs[slot].at[par, pl.ds(h * sk + vo, vn)], vsem.at[par, slot]).start(priority=1)
                ko += kn
                vo += vn

    def issue_w(gw_idx, piece):
        r = pl.multiple_of(piece * wrows, wrows)
        col = pl.multiple_of(gw_idx * gw, gw)
        for i, w in enumerate((wqa_hbm, wqb_hbm)):
            pltpu.make_async_copy(
                w.at[pl.ds(r, wrows), pl.ds(col, gw)],
                wq_buf.at[gw_idx, i, pl.ds(r, wrows)], wqsem.at[gw_idx]).start(priority=i)
        for i, w in enumerate((woa_hbm, wob_hbm)):
            pltpu.make_async_copy(
                w.at[pl.ds(col + r, wrows)],
                wo_buf.at[gw_idx, i, pl.ds(r, wrows)], wosem.at[gw_idx]).start(priority=i)

    def issue_packet(u, slot):
        gu = u // nb
        bu = u % nb
        issue_kv(gu, bu, slot, (u // bc) % NPAR)

        if not NOW:
            @pl.when(gu + 1 < hkv)
            def _():
                issue_w(gu + 1, bu)

    @pl.when(jnp.logical_and(g == 0, c == 0))
    def _():
        xr = 64
        for j in range(nb * sq // xr):
            for i, x in enumerate((xa_hbm, xb_hbm)):
                pltpu.make_async_copy(
                    x.at[pl.ds(j * xr, xr)], x_buf.at[i, pl.ds(j * xr, xr)], xsem.at[0]).start(priority=i)
        for j in range(nb):
            issue_w(0, j)
        for j in range(LA):
            issue_packet(j, j % bc)
        pltpu.make_async_copy(x_buf, x_buf, xsem.at[0]).wait()

    @pl.when(jnp.logical_and(c == 0, g * NOW == 0))
    def _():
        pltpu.make_async_copy(wq_buf.at[g], wq_buf.at[g], wqsem.at[g]).wait()

    xa = x_buf[0, pl.ds(r0, rows), :]
    qa = (jnp.dot(xa, wq_buf[g, 0], preferred_element_type=jnp.float32) * qscale).astype(jnp.bfloat16)
    xb = x_buf[1, pl.ds(r0, rows), :]
    qb = (jnp.dot(xb, wq_buf[g, 1], preferred_element_type=jnp.float32) * qscale).astype(jnp.bfloat16)

    par = (g * (nb // bc) + c) % NPAR

    def qk_unit(b):
        kb = kbufs[b].at[par]
        qab = jnp.concatenate(
            [qa[b * sq:(b + 1) * sq, r * dh:(r + 1) * dh] for r in range(rep)], axis=0)
        res = [_scores(qab, kb[0:sk, :])]
        for r in range(rep):
            res.append(_scores(qb[b * sq:(b + 1) * sq, r * dh:(r + 1) * dh],
                               kb[(r + 1) * sk:(r + 2) * sk, :]))
        return res

    def pv_unit(b, res):
        vb = vbufs[b].at[par]
        o = _pv(res[0][0], res[0][1], vb[0:sk, :])
        oa = jnp.concatenate([o[r * sq:(r + 1) * sq, :] for r in range(rep)], axis=1)
        ob = jnp.concatenate(
            [_pv(res[1 + r][0], res[1 + r][1], vb[(r + 1) * sk:(r + 2) * sk, :]) for r in range(rep)],
            axis=1)
        return oa, ob

    u0 = g * nb + c * bc
    outs = []
    for b in range(bc):
        un = u0 + b + LA
        slot_n = (b + LA) % bc

        if not ISSUE_FIRST:
            pltpu.make_async_copy(kbufs[b].at[par], kbufs[b].at[par], ksem.at[par, b]).wait()
            pltpu.make_async_copy(vbufs[b].at[par], vbufs[b].at[par], vsem.at[par, b]).wait()
        @pl.when(un < n_units)
        def _():
            issue_packet(un, slot_n)
        if ISSUE_FIRST:
            pltpu.make_async_copy(kbufs[b].at[par], kbufs[b].at[par], ksem.at[par, b]).wait()
            pltpu.make_async_copy(vbufs[b].at[par], vbufs[b].at[par], vsem.at[par, b]).wait()
        if NOCOMP:
            outs.append((qa[b * sq:(b + 1) * sq] + kbufs[b][par, 0:sq, 0:1], qb[b * sq:(b + 1) * sq] + vbufs[b][par, 0:sq, 0:1]))
        else:
            outs.append(pv_unit(b, qk_unit(b)))

    @pl.when(jnp.logical_and(c == 0, g * NOW == 0))
    def _():
        pltpu.make_async_copy(wo_buf.at[g], wo_buf.at[g], wosem.at[g]).wait()

    oa = jnp.concatenate([o[0] for o in outs], axis=0)
    ob = jnp.concatenate([o[1] for o in outs], axis=0)
    ya = jnp.dot(oa, wo_buf[g, 0], preferred_element_type=jnp.float32)
    yb = jnp.dot(ob, wo_buf[g, 1], preferred_element_type=jnp.float32)

    @pl.when(g == 0)
    def _():
        acc_ref[pl.ds(r0, rows), 0:d] = ya
        acc_ref[pl.ds(r0, rows), d:2 * d] = yb

    @pl.when(g > 0)
    def _():
        acc_ref[pl.ds(r0, rows), 0:d] += ya
        acc_ref[pl.ds(r0, rows), d:2 * d] += yb

    @pl.when(g == pl.num_programs(0) - 1)
    def _():
        out_ref[...] = acc_ref[pl.ds(r0, rows), :].astype(out_ref.dtype)


@jax.jit
def pallas_concat_heads__gqa_block_cached__mha_block_cached__near_ridge_kernel(
    A_x, A_k_cache, A_v_cache, A_wq, A_wo, B_x, B_k_cache, B_v_cache, B_wq, B_wo,
):
    B, Sq, D = A_x.shape
    _, Hkv, Sk, Dh = A_k_cache.shape
    H = B_k_cache.shape[1]
    rep = H // Hkv
    bc = 4
    nc = B // bc
    rows = bc * Sq
    gw = rep * Dh
    qscale = (Dh ** -0.5) * _LOG2E
    bf16 = A_x.dtype

    hbm = pl.BlockSpec(memory_space=pl.ANY)
    out_spec = pl.BlockSpec(
        (rows, 2 * D), lambda g, c: (jnp.where(g == Hkv - 1, c, 0), 0))
    kv_buf = pltpu.VMEM((NPAR, (rep + 1) * Sk, Dh), bf16)

    out = pl.pallas_call(
        functools.partial(_kernel, nb=B, bc=bc, sq=Sq, sk=Sk, dh=Dh, rep=rep, d=D, hkv=Hkv,
                          qscale=qscale),
        grid=(Hkv, nc),
        in_specs=[hbm] * 10,
        out_specs=out_spec,
        out_shape=jax.ShapeDtypeStruct((B * Sq, 2 * D), bf16),
        scratch_shapes=[
            pltpu.VMEM((B * Sq, 2 * D), jnp.float32),
            pltpu.VMEM((2, B * Sq, D), bf16),
            pltpu.VMEM((Hkv, 2, D, gw), bf16),
            pltpu.VMEM((Hkv, 2, gw, D), bf16),
        ] + [kv_buf] * (2 * bc) + [
            pltpu.SemaphoreType.DMA((NPAR, bc)),
            pltpu.SemaphoreType.DMA((NPAR, bc)),
            pltpu.SemaphoreType.DMA((Hkv,)),
            pltpu.SemaphoreType.DMA((Hkv,)),
            pltpu.SemaphoreType.DMA((1,)),
        ],
        compiler_params=pltpu.CompilerParams(
            dimension_semantics=("arbitrary", "arbitrary"),
            vmem_limit_bytes=64 * 1024 * 1024,
            disable_bounds_checks=bool(NOCHK),
        ),
    )(A_x.reshape(B * Sq, D), A_k_cache.reshape(-1, Dh), A_v_cache.reshape(-1, Dh), A_wq, A_wo,
      B_x.reshape(B * Sq, D), B_k_cache.reshape(-1, Dh), B_v_cache.reshape(-1, Dh), B_wq, B_wo)
    return out.reshape(B, Sq, 2 * D)
```

```python
import functools
import math

import jax
import jax.numpy as jnp
from jax import lax
import jax.experimental.pallas as pl
import jax.experimental.pallas.tpu as pltpu

_NT = (((1,), (1,)), ((), ()))
_LOG2E = math.log2(math.e)

_PHASE = 88
_K_CUTS = (0, 272)
_V_CUTS = (0, 256)
_W_PHASE = 24
_W_CUTS = ((72, 56), (64, 64))
_WQ_CUT = (11, 13)
_FINE = 2


def _softmax_parts(q, k):
    s = lax.dot_general(q, k, _NT, preferred_element_type=jnp.float32)
    m = jnp.max(s, axis=-1, keepdims=True)
    p = jnp.exp2(s - m)
    l = jnp.sum(p, axis=-1, keepdims=True)
    r = pl.reciprocal(l, approx=True)
    r = r * (2.0 - l * r)
    return p.astype(jnp.bfloat16), r


def _pv(p, r, v):
    o = jnp.dot(p, v, preferred_element_type=jnp.float32)
    return (o * r).astype(jnp.bfloat16)


def _packets(total, unit, cuts):
    bounds = sorted({0, total} | {_PHASE + 512 * j + c for j in range(total // 512) for c in cuts})
    packets = [[] for _ in range(total // unit)]
    for lo, hi in zip(bounds[:-1], bounds[1:]):
        packets[max(0, (lo - _PHASE) // unit)].append((lo, hi - lo))
    return packets


def _kernel(xa_hbm, ka_hbm, va_hbm, wqa_hbm, woa_hbm,
            xb_hbm, kb_hbm, vb_hbm, wqb_hbm, wob_hbm,
            out_hbm,
            o_buf, x_buf, wq_buf, wo_buf, q_buf, ka_all, va_all, kb_all, vb_all,
            ka_sems, va_sems, kb_sems, vb_sems, w_sems,
            *, nb, sq, sk, dh, rep, d, hkv, qscale):
    b = pl.program_id(0)
    gw = rep * dh
    a_rows = hkv * sk
    b_rows = hkv * rep * sk
    ka_p = _packets(a_rows, sk, _K_CUTS)
    va_p = _packets(a_rows, sk, _V_CUTS)
    kb_p = _packets(b_rows, rep * sk, _K_CUTS)
    vb_p = _packets(b_rows, rep * sk, _V_CUTS)

    def vb_slot(g, row):
        if g == hkv - 1:
            return g + (row - _PHASE - g * rep * sk) // sk
        return g

    def start_packet(bu, g):
        kc = ([(ka_hbm, ka_all, ka_sems, a_rows, o, r, g) for o, r in ka_p[g]]
              + [(kb_hbm, kb_all, kb_sems, b_rows, o, r, g) for o, r in kb_p[g]])
        vc = ([(va_hbm, va_all, va_sems, a_rows, o, r, g) for o, r in va_p[g]]
              + [(vb_hbm, vb_all, vb_sems, b_rows, o, r, vb_slot(g, o)) for o, r in vb_p[g]])
        slot = bu % 2
        for pair in zip(kc, vc):
            for priority, (src, dst, sems, n, o, r, s) in enumerate(pair):
                pltpu.make_async_copy(src.at[pl.ds(pl.multiple_of(bu * n + o, 8), r)],
                                      dst.at[slot, pl.ds(o, r)],
                                      sems.at[slot, s]).start(priority=priority)

    par = b % 2
    ka_buf, va_buf, kb_buf, vb_buf = (r.at[par] for r in (ka_all, va_all, kb_all, vb_all))
    ka_sem, va_sem, kb_sem, vb_sem = (r.at[par] for r in (ka_sems, va_sems, kb_sems, vb_sems))

    def wait_all(view, sem):
        pltpu.make_async_copy(view, view, sem).wait()

    def wait_rows(buf, pieces, sem):
        wait_all(buf.at[pl.ds(pieces[0][0], sum(r for _, r in pieces))], sem)

    def wait_k(g):
        wait_rows(ka_buf, ka_p[g], ka_sem.at[g])
        wait_rows(kb_buf, kb_p[g], kb_sem.at[g])

    def q_proj(bu, g):
        r0 = pl.multiple_of(bu * sq, sq)
        for i in range(2):
            q = (jnp.dot(x_buf[i, pl.ds(r0, sq), :], wq_buf[i, :, g * gw:(g + 1) * gw],
                         preferred_element_type=jnp.float32) * qscale).astype(jnp.bfloat16)
            for r in range(rep):
                q_buf[i, g, r * sq:(r + 1) * sq, :] = q[:, r * dh:(r + 1) * dh]

    @pl.when(b == 0)
    def _prologue():
        def stream_rows(srcs, dst, sem, total):
            per = sum(_W_CUTS[0])

            def piece(i, r, n):
                pltpu.make_async_copy(srcs[i].at[pl.ds(r, n)], dst.at[i, pl.ds(r, n)],
                                      sem).start(priority=i)

            def period(base, clip):
                offs = [_W_PHASE, _W_PHASE]
                for ns in zip(*_W_CUTS):
                    for i, n in enumerate(ns):
                        if clip:
                            piece(i, base + offs[i], min(n, per - offs[i]))
                        else:
                            piece(i, pl.multiple_of(base + offs[i], 8), n)
                        offs[i] += n

            for i in range(2):
                piece(i, 0, _W_PHASE)
            period(total - per, True)

            def body(j, carry):
                period(j * per, False)
                return carry
            lax.fori_loop(0, total // per - 1, body, 0)

        def wq_piece(i, slab, t0, t1):
            rows = pl.ds(pl.multiple_of(slab * 8, 8), 8)
            cols = pl.ds(t0 * 128, (t1 - t0) * 128)
            pltpu.make_async_copy((wqa_hbm, wqb_hbm)[i].at[rows, cols], wq_buf.at[i, rows, cols],
                                  w_sems.at[1]).start(priority=i)

        nt = hkv * gw // 128
        ns = d // 8
        c0, c1 = _WQ_CUT

        def wq_pair(s, last):
            wq_piece(0, s, c0, nt)
            wq_piece(0, s + 1, 0, c1)
            wq_piece(1, s, c0, nt)
            wq_piece(1, s + 1, 0, c0)
            wq_piece(0, s + 1, c1, nt)
            if not last:
                wq_piece(0, s + 2, 0, c0)
            wq_piece(1, s + 1, c0, nt)
            if not last:
                wq_piece(1, s + 2, 0, c0)

        def wq_body(j, carry):
            wq_pair(2 * j, False)
            return carry

        stream_rows((xa_hbm, xb_hbm), x_buf, w_sems.at[0], nb * sq)
        wq_piece(0, 0, 0, c0)
        wq_piece(1, 0, 0, c0)
        wq_pair(ns - 2, True)
        lax.fori_loop(0, ns // 2 - 1, wq_body, 0)
        stream_rows((woa_hbm, wob_hbm), wo_buf, w_sems.at[2], hkv * gw)
        start_packet(0, 0)
        wait_all(x_buf, w_sems.at[0])
        wait_all(wq_buf, w_sems.at[1])
        for g in range(hkv):
            if g + 1 < hkv:
                start_packet(0, g + 1)
            q_proj(0, g)
            wait_all(wo_buf.at[:, pl.ds(g * gw, gw)], w_sems.at[2])

    def qk_unit(g):
        res = [_softmax_parts(q_buf[0, g], ka_buf[g * sk:(g + 1) * sk, :])]
        for r in range(rep):
            h = g * rep + r
            res.append(_softmax_parts(q_buf[1, g, r * sq:(r + 1) * sq, :],
                                      kb_buf[h * sk:(h + 1) * sk, :]))
        return res

    def pv_unit(g, res):
        o = _pv(*res[0], va_buf[g * sk:(g + 1) * sk, :])
        oa = jnp.concatenate([o[r * sq:(r + 1) * sq, :] for r in range(rep)], axis=1)
        ob = jnp.concatenate(
            [_pv(*res[1 + r], vb_buf[(g * rep + r) * sk:(g * rep + r + 1) * sk, :])
             for r in range(rep)], axis=1)
        return oa, ob

    def out_proj(g, o, y):
        z = [jnp.dot(o[i], wo_buf[i, g * gw:(g + 1) * gw, :], preferred_element_type=jnp.float32)
             for i in range(2)]
        return z if y is None else [z[0] + y[0], z[1] + y[1]]

    def store_rows(r, priority):
        pltpu.make_async_copy(o_buf.at[pl.ds(r, sq)], out_hbm.at[pl.ds(r, sq)],
                              w_sems.at[0]).start(priority=priority)

    y = None
    wait_k(0)
    res = qk_unit(0)
    for g in range(hkv):
        if g + 1 < hkv:
            wait_k(g + 1)
        wait_rows(va_buf, va_p[g], va_sem.at[g])
        for s in sorted({vb_slot(g, o) for o, _ in vb_p[g]}):
            if s == hkv - 2 + _FINE:
                @pl.when(b == nb - 1)
                def _():
                    for j in range(nb - 1):
                        store_rows(j * sq, 1)
            wait_rows(vb_buf, [p for p in vb_p[g] if vb_slot(g, p[0]) == s], vb_sem.at[s])

        @pl.when(b + 1 < nb)
        def _():
            start_packet(b + 1, g)

        @pl.when(b < nb - 1)
        def _():
            q_proj(b + 1, g)

        o = pv_unit(g, res)
        if g + 1 < hkv:
            res = qk_unit(g + 1)
        y = out_proj(g, o, y)

    r0 = pl.multiple_of(b * sq, sq)
    o_buf[pl.ds(r0, sq), 0:d] = y[0].astype(o_buf.dtype)
    o_buf[pl.ds(r0, sq), d:2 * d] = y[1].astype(o_buf.dtype)

    @pl.when(b == nb - 1)
    def _():
        store_rows((nb - 1) * sq, 0)
        pltpu.make_async_copy(o_buf, out_hbm, w_sems.at[0]).wait()


@jax.jit
def pallas_concat_heads__gqa_block_cached__mha_block_cached__near_ridge_kernel(
    A_x, A_k_cache, A_v_cache, A_wq, A_wo, B_x, B_k_cache, B_v_cache, B_wq, B_wo,
):
    B, Sq, D = A_x.shape
    _, Hkv, Sk, Dh = A_k_cache.shape
    H = B_k_cache.shape[1]
    rep = H // Hkv
    qscale = (Dh ** -0.5) * _LOG2E
    dt = A_x.dtype

    hbm = pl.BlockSpec(memory_space=pl.ANY)
    out = pl.pallas_call(
        functools.partial(_kernel, nb=B, sq=Sq, sk=Sk, dh=Dh, rep=rep, d=D, hkv=Hkv, qscale=qscale),
        grid=(B,),
        in_specs=[hbm] * 10,
        out_specs=hbm,
        out_shape=jax.ShapeDtypeStruct((B * Sq, 2 * D), dt),
        scratch_shapes=[
            pltpu.VMEM((B * Sq, 2 * D), dt),
            pltpu.VMEM((2, B * Sq, D), dt),
            pltpu.VMEM((2, D, H * Dh), dt),
            pltpu.VMEM((2, H * Dh, D), dt),
            pltpu.VMEM((2, Hkv, rep * Sq, Dh), dt),
            pltpu.VMEM((2, Hkv * Sk, Dh), dt),
            pltpu.VMEM((2, Hkv * Sk, Dh), dt),
            pltpu.VMEM((2, H * Sk, Dh), dt),
            pltpu.VMEM((2, H * Sk, Dh), dt),
            pltpu.SemaphoreType.DMA((2, Hkv)),
            pltpu.SemaphoreType.DMA((2, Hkv)),
            pltpu.SemaphoreType.DMA((2, Hkv)),
            pltpu.SemaphoreType.DMA((2, Hkv + rep - 1)),
            pltpu.SemaphoreType.DMA((3,)),
        ],
        compiler_params=pltpu.CompilerParams(
            dimension_semantics=("arbitrary",),
            vmem_limit_bytes=64 * 1024 * 1024,
            disable_bounds_checks=True,
            disable_semaphore_checks=True,
        ),
    )(A_x.reshape(B * Sq, D), A_k_cache.reshape(-1, Dh), A_v_cache.reshape(-1, Dh), A_wq, A_wo,
      B_x.reshape(B * Sq, D), B_k_cache.reshape(-1, Dh), B_v_cache.reshape(-1, Dh), B_wq, B_wo)
    return out.reshape(B, Sq, 2 * D)
```

```python
import functools
import math

import jax
import jax.numpy as jnp
from jax import lax
import jax.experimental.pallas as pl
import jax.experimental.pallas.tpu as pltpu

_NT = (((1,), (1,)), ((), ()))
_LOG2E = math.log2(math.e)

_PHASE = 88
_K_CUTS = (0, 272)
_V_CUTS = (0, 256)
_W_PHASE = 24
_W_CUTS = ((72, 56), (64, 64))
_WQ_CUT = (11, 13)
_FINE = 2


def _softmax_parts(q, k):
    s = lax.dot_general(q, k, _NT, preferred_element_type=jnp.float32)
    m = jnp.max(s, axis=-1, keepdims=True)
    p = jnp.exp2(s - m)
    l = jnp.sum(p, axis=-1, keepdims=True)
    r = pl.reciprocal(l, approx=True)
    r = r * (2.0 - l * r)
    return p.astype(jnp.bfloat16), r


def _pv(p, r, v):
    o = jnp.dot(p, v, preferred_element_type=jnp.float32)
    return (o * r).astype(jnp.bfloat16)


def _packets(total, unit, cuts):
    bounds = sorted({0, total} | {_PHASE + 512 * j + c for j in range(total // 512) for c in cuts})
    packets = [[] for _ in range(total // unit)]
    for lo, hi in zip(bounds[:-1], bounds[1:]):
        packets[max(0, (lo - _PHASE) // unit)].append((lo, hi - lo))
    return packets


def _kernel(xa_hbm, ka_hbm, va_hbm, wqa_hbm, woa_hbm,
            xb_hbm, kb_hbm, vb_hbm, wqb_hbm, wob_hbm,
            out_hbm,
            o_buf, x_buf, wq_buf, wo_buf, q_buf, ka_all, va_all, kb_all, vb_all,
            ka_sems, va_sems, kb_sems, vb_sems, w_sems,
            *, nb, sq, sk, dh, rep, d, hkv, qscale):
    b = pl.program_id(0)
    gw = rep * dh
    a_rows = hkv * sk
    b_rows = hkv * rep * sk
    ka_p = _packets(a_rows, sk, _K_CUTS)
    va_p = _packets(a_rows, sk, _V_CUTS)
    kb_p = _packets(b_rows, rep * sk, _K_CUTS)
    vb_p = _packets(b_rows, rep * sk, _V_CUTS)

    def vb_slot(g, row):
        if g == hkv - 1:
            return g + (row - _PHASE - g * rep * sk) // sk
        return g

    def start_packet(bu, g):
        kc = ([(ka_hbm, ka_all, ka_sems, a_rows, o, r, g) for o, r in ka_p[g]]
              + [(kb_hbm, kb_all, kb_sems, b_rows, o, r, g) for o, r in kb_p[g]])
        vc = ([(va_hbm, va_all, va_sems, a_rows, o, r, g) for o, r in va_p[g]]
              + [(vb_hbm, vb_all, vb_sems, b_rows, o, r, vb_slot(g, o)) for o, r in vb_p[g]])
        slot = bu % 2
        for pair in zip(kc, vc):
            for priority, (src, dst, sems, n, o, r, s) in enumerate(pair):
                pltpu.make_async_copy(src.at[pl.ds(pl.multiple_of(bu * n + o, 8), r)],
                                      dst.at[slot, pl.ds(o, r)],
                                      sems.at[slot, s]).start(priority=priority)

    par = b % 2
    ka_buf, va_buf, kb_buf, vb_buf = (r.at[par] for r in (ka_all, va_all, kb_all, vb_all))
    ka_sem, va_sem, kb_sem, vb_sem = (r.at[par] for r in (ka_sems, va_sems, kb_sems, vb_sems))

    def wait_all(view, sem):
        pltpu.make_async_copy(view, view, sem).wait()

    def wait_rows(buf, pieces, sem):
        wait_all(buf.at[pl.ds(pieces[0][0], sum(r for _, r in pieces))], sem)

    def wait_k(g):
        wait_rows(ka_buf, ka_p[g], ka_sem.at[g])
        wait_rows(kb_buf, kb_p[g], kb_sem.at[g])

    def q_proj(bu, g):
        r0 = pl.multiple_of(bu * sq, sq)
        for i in range(2):
            q = (jnp.dot(x_buf[i, pl.ds(r0, sq), :], wq_buf[i, :, g * gw:(g + 1) * gw],
                         preferred_element_type=jnp.float32) * qscale).astype(jnp.bfloat16)
            for r in range(rep):
                q_buf[i, g, r * sq:(r + 1) * sq, :] = q[:, r * dh:(r + 1) * dh]

    @pl.when(b == 0)
    def _prologue():
        per = sum(_W_CUTS[0])

        def stream_rows(srcs, dst, sem_of, total):
            def piece(i, j, r, n):
                pltpu.make_async_copy(srcs[i].at[pl.ds(r, n)], dst.at[i, pl.ds(r, n)],
                                      w_sems.at[sem_of(i, j)]).start(priority=i)

            def period(j, clip):
                offs = [_W_PHASE, _W_PHASE]
                for sizes in zip(*_W_CUTS):
                    for i, n in enumerate(sizes):
                        piece(i, j, pl.multiple_of(j * per + offs[i], 8),
                              min(n, per - offs[i]) if clip else n)
                        offs[i] += n

            for i in range(2):
                piece(i, 0, 0, _W_PHASE)
            period(total // per - 1, True)

            def body(j, carry):
                period(j, False)
                return carry
            lax.fori_loop(0, total // per - 1, body, 0)

        def wq_piece(i, slab, t0, t1):
            rows = pl.ds(pl.multiple_of(slab * 8, 8), 8)
            cols = pl.ds(t0 * 128, (t1 - t0) * 128)
            pltpu.make_async_copy((wqa_hbm, wqb_hbm)[i].at[rows, cols], wq_buf.at[i, rows, cols],
                                  w_sems.at[1]).start(priority=i)

        nt = hkv * gw // 128
        ns = d // 8
        c0, c1 = _WQ_CUT

        def wq_pair(s, last):
            wq_piece(0, s, c0, nt)
            wq_piece(0, s + 1, 0, c1)
            wq_piece(1, s, c0, nt)
            wq_piece(1, s + 1, 0, c0)
            wq_piece(0, s + 1, c1, nt)
            if not last:
                wq_piece(0, s + 2, 0, c0)
            wq_piece(1, s + 1, c0, nt)
            if not last:
                wq_piece(1, s + 2, 0, c0)

        def wq_body(j, carry):
            wq_pair(2 * j, False)
            return carry

        stream_rows((xa_hbm, xb_hbm), x_buf, lambda i, j: 0, nb * sq)
        wq_piece(0, 0, 0, c0)
        wq_piece(1, 0, 0, c0)
        wq_pair(ns - 2, True)
        lax.fori_loop(0, ns // 2 - 1, wq_body, 0)
        stream_rows((woa_hbm, wob_hbm), wo_buf,
                    lambda i, j: 2 if i else 3 + lax.div(j, gw // per), hkv * gw)
        start_packet(0, 0)
        wait_all(x_buf, w_sems.at[0])
        wait_all(wq_buf, w_sems.at[1])
        for g in range(hkv):
            if g + 1 < hkv:
                start_packet(0, g + 1)
            q_proj(0, g)
            lo = g * gw + _W_PHASE if g else 0
            hi = min((g + 1) * gw + _W_PHASE, hkv * gw)
            wait_all(wo_buf.at[0, pl.ds(lo, hi - lo)], w_sems.at[3 + g])
        wait_all(wo_buf.at[1], w_sems.at[2])

    def qk_unit(g):
        res = [_softmax_parts(q_buf[0, g], ka_buf[g * sk:(g + 1) * sk, :])]
        for r in range(rep):
            h = g * rep + r
            res.append(_softmax_parts(q_buf[1, g, r * sq:(r + 1) * sq, :],
                                      kb_buf[h * sk:(h + 1) * sk, :]))
        return res

    def pv_unit(g, res):
        o = _pv(*res[0], va_buf[g * sk:(g + 1) * sk, :])
        oa = jnp.concatenate([o[r * sq:(r + 1) * sq, :] for r in range(rep)], axis=1)
        ob = jnp.concatenate(
            [_pv(*res[1 + r], vb_buf[(g * rep + r) * sk:(g * rep + r + 1) * sk, :])
             for r in range(rep)], axis=1)
        return oa, ob

    def out_proj(g, o, y):
        z = [jnp.dot(o[i], wo_buf[i, g * gw:(g + 1) * gw, :], preferred_element_type=jnp.float32)
             for i in range(2)]
        return z if y is None else [z[0] + y[0], z[1] + y[1]]

    def store_rows(r, priority):
        pltpu.make_async_copy(o_buf.at[pl.ds(r, sq)], out_hbm.at[pl.ds(r, sq)],
                              w_sems.at[0]).start(priority=priority)

    y = None
    wait_k(0)
    res = qk_unit(0)
    for g in range(hkv):
        if g + 1 < hkv:
            wait_k(g + 1)
        wait_rows(va_buf, va_p[g], va_sem.at[g])
        for s in sorted({vb_slot(g, o) for o, _ in vb_p[g]}):
            if s == hkv - 2 + _FINE:
                @pl.when(b == nb - 1)
                def _():
                    for j in range(nb - 1):
                        store_rows(j * sq, 1)
            wait_rows(vb_buf, [p for p in vb_p[g] if vb_slot(g, p[0]) == s], vb_sem.at[s])

        @pl.when(b + 1 < nb)
        def _():
            start_packet(b + 1, g)

        @pl.when(b < nb - 1)
        def _():
            q_proj(b + 1, g)

        o = pv_unit(g, res)
        if g + 1 < hkv:
            res = qk_unit(g + 1)
        y = out_proj(g, o, y)

    r0 = pl.multiple_of(b * sq, sq)
    o_buf[pl.ds(r0, sq), 0:d] = y[0].astype(o_buf.dtype)
    o_buf[pl.ds(r0, sq), d:2 * d] = y[1].astype(o_buf.dtype)

    @pl.when(b == nb - 1)
    def _():
        store_rows((nb - 1) * sq, 0)
        pltpu.make_async_copy(o_buf, out_hbm, w_sems.at[0]).wait()


@jax.jit
def pallas_concat_heads__gqa_block_cached__mha_block_cached__near_ridge_kernel(
    A_x, A_k_cache, A_v_cache, A_wq, A_wo, B_x, B_k_cache, B_v_cache, B_wq, B_wo,
):
    B, Sq, D = A_x.shape
    _, Hkv, Sk, Dh = A_k_cache.shape
    H = B_k_cache.shape[1]
    rep = H // Hkv
    qscale = (Dh ** -0.5) * _LOG2E
    dt = A_x.dtype

    hbm = pl.BlockSpec(memory_space=pl.ANY)
    out = pl.pallas_call(
        functools.partial(_kernel, nb=B, sq=Sq, sk=Sk, dh=Dh, rep=rep, d=D, hkv=Hkv, qscale=qscale),
        grid=(B,),
        in_specs=[hbm] * 10,
        out_specs=hbm,
        out_shape=jax.ShapeDtypeStruct((B * Sq, 2 * D), dt),
        scratch_shapes=[
            pltpu.VMEM((B * Sq, 2 * D), dt),
            pltpu.VMEM((2, B * Sq, D), dt),
            pltpu.VMEM((2, D, H * Dh), dt),
            pltpu.VMEM((2, H * Dh, D), dt),
            pltpu.VMEM((2, Hkv, rep * Sq, Dh), dt),
            pltpu.VMEM((2, Hkv * Sk, Dh), dt),
            pltpu.VMEM((2, Hkv * Sk, Dh), dt),
            pltpu.VMEM((2, H * Sk, Dh), dt),
            pltpu.VMEM((2, H * Sk, Dh), dt),
            pltpu.SemaphoreType.DMA((2, Hkv)),
            pltpu.SemaphoreType.DMA((2, Hkv)),
            pltpu.SemaphoreType.DMA((2, Hkv)),
            pltpu.SemaphoreType.DMA((2, Hkv + rep - 1)),
            pltpu.SemaphoreType.DMA((3 + Hkv,)),
        ],
        compiler_params=pltpu.CompilerParams(
            dimension_semantics=("arbitrary",),
            vmem_limit_bytes=64 * 1024 * 1024,
            disable_bounds_checks=True,
            disable_semaphore_checks=True,
        ),
    )(A_x.reshape(B * Sq, D), A_k_cache.reshape(-1, Dh), A_v_cache.reshape(-1, Dh), A_wq, A_wo,
      B_x.reshape(B * Sq, D), B_k_cache.reshape(-1, Dh), B_v_cache.reshape(-1, Dh), B_wq, B_wo)
    return out.reshape(B, Sq, 2 * D)
```

```python
import functools
import math

import jax
import jax.numpy as jnp
from jax import lax
import jax.experimental.pallas as pl
import jax.experimental.pallas.tpu as pltpu

_NT = (((1,), (1,)), ((), ()))
_LOG2E = math.log2(math.e)

_STRIPE = 256
_CUTS = ((96, 104), (104, 88, 104, 96, 112, 104, 96, 104),
         (96, 88), (80, 96, 80, 88, 88, 88, 88, 88))
_ORDER = (2, 0, 3, 4, 5, 6, 7, 8, 1, 9)
_PAD = 128
_LOOKAHEAD = 6
_TRIGGER = 4
_X_ROWS = 32
_W_PHASE = 24
_W_PERIOD = 128
_WO_CUT = 2 * 128
_WQ_CUT = (11, 13)


def _softmax_parts(q, k):
    s = lax.dot_general(q, k, _NT, preferred_element_type=jnp.float32)
    m = jnp.max(s, axis=-1, keepdims=True)
    p = jnp.exp2(s - m)
    l = jnp.sum(p, axis=-1, keepdims=True)
    r = pl.reciprocal(l, approx=True)
    r = r * (2.0 - l * r)
    return p.astype(jnp.bfloat16), r


def _pv(p, r, v):
    o = jnp.dot(p, v, preferred_element_type=jnp.float32)
    return (o * r).astype(jnp.bfloat16)


def _kernel(xa_hbm, ka_hbm, va_hbm, wqa_hbm, woa_hbm,
            xb_hbm, kb_hbm, vb_hbm, wqb_hbm, wob_hbm,
            out_hbm,
            o_buf, x_buf, wq_buf, wo_buf, q_buf, kv_all, k_sems, v_sems, w_sems,
            *, nb, sq, sk, dh, rep, d, hkv, qscale):
    b = pl.program_id(0)
    gw = rep * dh
    last = hkv - 1
    srcs = (ka_hbm, kb_hbm, va_hbm, vb_hbm)
    unit = (sk, rep * sk, sk, rep * sk)
    rows = tuple(hkv * u for u in unit)
    base = tuple(sum(rows[:s]) + s * _PAD for s in range(4))

    def pieces(s, g, clip):
        c = [g * unit[s] + j * _STRIPE + o for j, o in enumerate(_CUTS[s] + _CUTS[s][:1])]
        if clip:
            c[-1] = rows[s]
        return [(s, lo, hi - lo) for lo, hi in zip(c[:-1], c[1:])]

    def sequence(v, g, clip):
        pcs = pieces(2 * v, g, clip) + pieces(2 * v + 1, g, clip)
        return [pcs[i] for i in _ORDER]

    def sem_slot(v, g, i):
        return hkv if (v and g == last and i < _TRIGGER) else g

    def start_packet(bu, g, clip):
        slot = bu % 2
        for i, pair in enumerate(zip(sequence(0, g, clip), sequence(1, g, clip))):
            for v, (s, lo, n) in enumerate(pair):
                pltpu.make_async_copy(srcs[s].at[pl.ds(pl.multiple_of(bu * rows[s] + lo, 8), n)],
                                      kv_all.at[slot, pl.ds(base[s] + lo, n)],
                                      (k_sems, v_sems)[v].at[slot, sem_slot(v, g, i)]).start(priority=v)

    par = b % 2
    kv = kv_all.at[par]

    def wait_all(view, sem):
        pltpu.make_async_copy(view, view, sem).wait()

    def wait_slot(v, slot, clip):
        g = min(slot, last)
        pcs = sorted(p for i, p in enumerate(sequence(v, g, clip)) if sem_slot(v, g, i) == slot)
        runs = []
        for s, lo, n in pcs:
            if runs and runs[-1][0] == s and runs[-1][1] + runs[-1][2] == lo:
                runs[-1][2] += n
            else:
                runs.append([s, lo, n])
        for s, lo, n in runs:
            wait_all(kv.at[pl.ds(base[s] + lo, n)], (k_sems, v_sems)[v].at[par, slot])

    def wait_kv(v, g):
        if g < last:
            wait_slot(v, g, False)
        else:
            pl.when(b < nb - 1)(lambda: wait_slot(v, g, False))
            pl.when(b == nb - 1)(lambda: wait_slot(v, g, True))

    def q_proj(bu, g):
        r0 = pl.multiple_of(bu * sq, sq)
        for i in range(2):
            q = (jnp.dot(x_buf[i, pl.ds(r0, sq), :], wq_buf[i, :, g * gw:(g + 1) * gw],
                         preferred_element_type=jnp.float32) * qscale).astype(jnp.bfloat16)
            for r in range(rep):
                q_buf[i, g, r * sq:(r + 1) * sq, :] = q[:, r * dh:(r + 1) * dh]

    @pl.when(b == 0)
    def _prologue():
        def x_piece(i, r, n):
            pltpu.make_async_copy((xa_hbm, xb_hbm)[i].at[pl.ds(r, n)], x_buf.at[i, pl.ds(r, n)],
                                  w_sems.at[0]).start(priority=1)

        def x_body(j, carry):
            for i in range(2):
                x_piece(i, pl.multiple_of(j * _X_ROWS + _W_PHASE, 8), _X_ROWS)
            return carry

        def wq_piece(i, slab, t0, t1):
            rws = pl.ds(pl.multiple_of(slab * 8, 8), 8)
            cols = pl.ds(t0 * 128, (t1 - t0) * 128)
            pltpu.make_async_copy((wqa_hbm, wqb_hbm)[i].at[rws, cols], wq_buf.at[i, rws, cols],
                                  w_sems.at[1]).start(priority=i)

        nt = hkv * gw // 128
        ns = d // 8
        c0, c1 = _WQ_CUT

        def wq_pair(s, is_last):
            wq_piece(0, s, c0, nt)
            wq_piece(0, s + 1, 0, c1)
            wq_piece(1, s, c0, nt)
            wq_piece(1, s + 1, 0, c0)
            wq_piece(0, s + 1, c1, nt)
            if not is_last:
                wq_piece(0, s + 2, 0, c0)
            wq_piece(1, s + 1, c0, nt)
            if not is_last:
                wq_piece(1, s + 2, 0, c0)

        def wq_body(j, carry):
            wq_pair(2 * j, False)
            return carry

        def wo_piece(i, j, r, n, cols=None):
            idx = (pl.ds(r, n),) if cols is None else (pl.ds(r, n), pl.ds(*cols))
            sem = 2 if i else 4 + lax.div(j, gw // _W_PERIOD)
            pltpu.make_async_copy((woa_hbm, wob_hbm)[i].at[idx], wo_buf.at[(i,) + idx],
                                  w_sems.at[sem]).start(priority=i)

        def wo_period(j, clip):
            r = lambda o: pl.multiple_of(j * _W_PERIOD + _W_PHASE + o, 8)
            wo_piece(0, j, r(0), 64)
            wo_piece(0, j, r(64), 8, (0, _WO_CUT))
            wo_piece(1, j, r(0), 64)
            wo_piece(0, j, r(64), 8, (_WO_CUT, d - _WO_CUT))
            wo_piece(0, j, r(72), 56 - clip)
            wo_piece(1, j, r(64), 64 - clip)

        def wo_body(j, carry):
            wo_period(j, 0)
            return carry

        def head_rows(s):
            return kv_all.at[0, pl.ds(base[s], _CUTS[s][0])]

        for i in range(2):
            x_piece(i, 0, _W_PHASE)
            x_piece(i, nb * sq - _X_ROWS + _W_PHASE, _X_ROWS - _W_PHASE)
        for s in (0, 2, 1, 3):
            pltpu.make_async_copy(srcs[s].at[pl.ds(0, _CUTS[s][0])], head_rows(s),
                                  w_sems.at[3]).start(priority=0)
        lax.fori_loop(0, nb * sq // _X_ROWS - 1, x_body, 0)
        wq_piece(0, 0, 0, c0)
        wq_piece(1, 0, 0, c0)
        wq_pair(ns - 2, True)
        lax.fori_loop(0, ns // 2 - 1, wq_body, 0)
        for i in range(2):
            wo_piece(i, 0, 0, _W_PHASE)
        wo_period(hkv * gw // _W_PERIOD - 1, _W_PHASE)
        lax.fori_loop(0, hkv * gw // _W_PERIOD - 1, wo_body, 0)
        start_packet(0, 0, False)
        wait_all(x_buf, w_sems.at[0])
        wait_all(wq_buf, w_sems.at[1])
        for g in range(hkv):
            if g + 1 < _LOOKAHEAD:
                start_packet(0, g + 1, False)
            q_proj(0, g)
            lo = g * gw + _W_PHASE if g else 0
            hi = min((g + 1) * gw + _W_PHASE, hkv * gw)
            wait_all(wo_buf.at[0, pl.ds(lo, hi - lo)], w_sems.at[4 + g])
        wait_all(wo_buf.at[1], w_sems.at[2])
        for s in range(4):
            wait_all(head_rows(s), w_sems.at[3])

    def head(s, h):
        return kv[base[s] + h * sk:base[s] + (h + 1) * sk, :]

    def qk_unit(g):
        return ([_softmax_parts(q_buf[0, g], head(0, g))]
                + [_softmax_parts(q_buf[1, g, r * sq:(r + 1) * sq, :], head(1, g * rep + r))
                   for r in range(rep)])

    def pv_unit(g, res):
        o = _pv(*res[0], head(2, g))
        oa = jnp.concatenate([o[r * sq:(r + 1) * sq, :] for r in range(rep)], axis=1)
        ob = jnp.concatenate([_pv(*res[1 + r], head(3, g * rep + r)) for r in range(rep)], axis=1)
        return oa, ob

    def out_proj(g, o, y):
        z = [jnp.dot(o[i], wo_buf[i, g * gw:(g + 1) * gw, :], preferred_element_type=jnp.float32)
             for i in range(2)]
        return z if y is None else [z[0] + y[0], z[1] + y[1]]

    def store_rows(r, n, priority):
        pltpu.make_async_copy(o_buf.at[pl.ds(r, n)], out_hbm.at[pl.ds(r, n)],
                              w_sems.at[0]).start(priority=priority)

    y = None
    wait_kv(0, 0)
    res = qk_unit(0)
    for g in range(hkv):
        if g < last:
            wait_kv(0, g + 1)
        else:
            pl.when(b < nb - 1)(lambda: wait_slot(1, hkv, False))
        wait_kv(1, g)

        bu, gu = b + (g + _LOOKAHEAD) // hkv, (g + _LOOKAHEAD) % hkv
        if gu < last:
            pl.when(bu < nb)(lambda: start_packet(bu, gu, False))
        else:
            pl.when(bu < nb - 1)(lambda: start_packet(bu, gu, False))
            pl.when(bu == nb - 1)(lambda: start_packet(bu, gu, True))

        @pl.when(b < nb - 1)
        def _():
            q_proj(b + 1, g)
            if g == last:
                for s in range(4):
                    n = _CUTS[s][0]
                    kv_all[1 - par, base[s]:base[s] + n, :] = kv[base[s] + rows[s]:base[s] + rows[s] + n, :]

        o = pv_unit(g, res)
        if g == last - 1:
            @pl.when(b == nb - 1)
            def _():
                wait_slot(1, hkv, True)
                store_rows(0, (nb - 1) * sq, 1)
        if g < last:
            res = qk_unit(g + 1)
        y = out_proj(g, o, y)

    r0 = pl.multiple_of(b * sq, sq)
    o_buf[pl.ds(r0, sq), 0:d] = y[0].astype(o_buf.dtype)
    o_buf[pl.ds(r0, sq), d:2 * d] = y[1].astype(o_buf.dtype)

    @pl.when(b == nb - 1)
    def _():
        store_rows((nb - 1) * sq, sq, 0)
        pltpu.make_async_copy(o_buf, out_hbm, w_sems.at[0]).wait()


@jax.jit
def pallas_concat_heads__gqa_block_cached__mha_block_cached__near_ridge_kernel(
    A_x, A_k_cache, A_v_cache, A_wq, A_wo, B_x, B_k_cache, B_v_cache, B_wq, B_wo,
):
    B, Sq, D = A_x.shape
    _, Hkv, Sk, Dh = A_k_cache.shape
    H = B_k_cache.shape[1]
    rep = H // Hkv
    qscale = (Dh ** -0.5) * _LOG2E
    dt = A_x.dtype
    assert Sk == _STRIPE * len(_CUTS[0]) and rep * Sk == _STRIPE * len(_CUTS[1]) and B >= 2

    hbm = pl.BlockSpec(memory_space=pl.ANY)
    out = pl.pallas_call(
        functools.partial(_kernel, nb=B, sq=Sq, sk=Sk, dh=Dh, rep=rep, d=D, hkv=Hkv, qscale=qscale),
        grid=(B,),
        in_specs=[hbm] * 10,
        out_specs=hbm,
        out_shape=jax.ShapeDtypeStruct((B * Sq, 2 * D), dt),
        scratch_shapes=[
            pltpu.VMEM((B * Sq, 2 * D), dt),
            pltpu.VMEM((2, B * Sq, D), dt),
            pltpu.VMEM((2, D, H * Dh), dt),
            pltpu.VMEM((2, H * Dh, D), dt),
            pltpu.VMEM((2, Hkv, rep * Sq, Dh), dt),
            pltpu.VMEM((2, 2 * (Hkv + H) * Sk + 4 * _PAD, Dh), dt),
            pltpu.SemaphoreType.DMA((2, Hkv)),
            pltpu.SemaphoreType.DMA((2, Hkv + 1)),
            pltpu.SemaphoreType.DMA((4 + Hkv,)),
        ],
        compiler_params=pltpu.CompilerParams(
            dimension_semantics=("arbitrary",),
            vmem_limit_bytes=64 * 1024 * 1024,
            disable_bounds_checks=True,
            disable_semaphore_checks=True,
        ),
    )(A_x.reshape(B * Sq, D), A_k_cache.reshape(-1, Dh), A_v_cache.reshape(-1, Dh), A_wq, A_wo,
      B_x.reshape(B * Sq, D), B_k_cache.reshape(-1, Dh), B_v_cache.reshape(-1, Dh), B_wq, B_wo)
    return out.reshape(B, Sq, 2 * D)
```

```python
import functools
import math
import os

import jax
import jax.numpy as jnp
from jax import lax
import jax.experimental.pallas as pl
import jax.experimental.pallas.tpu as pltpu

_NT = (((1,), (1,)), ((), ()))
_LOG2E = math.log2(math.e)

E = lambda k, v: int(os.environ.get(k, v))
_lst = lambda k, v: tuple(int(x) for x in os.environ.get(k, v).split(','))
PH = E('PH', '104')
A_S = _lst('A_S', '128,128')
B_S = _lst('B_S', '32')
TRIG = E('TRIG', '7')
LA = E('LA', '3')
NOCOMP = E('NOCOMP', '0')
NB = E('NB', '16')
XM = E('XM', '0')
XP = E('XP', '32')
WOX = E('WOX', '0')
WQT = E('WQT', '13')
RR = E('RR', '4')
PACE = E('PACE', '1')
WR = E('WR', '1')


def _softmax_parts(q, k):
    s = lax.dot_general(q, k, _NT, preferred_element_type=jnp.float32)
    m = jnp.max(s, axis=-1, keepdims=True)
    p = jnp.exp2(s - m)
    l = jnp.sum(p, axis=-1, keepdims=True)
    r = pl.reciprocal(l, approx=True)
    r = r * (2.0 - l * r)
    return p.astype(jnp.bfloat16), r


def _pv(p, r, v):
    o = jnp.dot(p, v, preferred_element_type=jnp.float32)
    return (o * r).astype(jnp.bfloat16)


def _kernel(xa_hbm, ka_hbm, va_hbm, wqa_hbm, woa_hbm,
            xb_hbm, kb_hbm, vb_hbm, wqb_hbm, wob_hbm,
            out_hbm,
            o_buf, x_buf, wq_buf, wo_buf, q_buf, kv_all, k_sems, v_sems, w_sems,
            *, nb, sq, sk, dh, rep, d, hkv, qscale):
    b = pl.program_id(0)
    gw = rep * dh
    last = hkv - 1
    rows = hkv * sk
    sems = (k_sems, v_sems)

    def cut(t, lo, sizes):
        sizes = sizes * (256 // sum(sizes))
        c = [lo + sum(sizes[:i]) for i in range(len(sizes) + 1)]
        pcs = [(t, max(x, 0), min(y, rows) - max(x, 0)) for x, y in zip(c[:-1], c[1:])]
        return [p for p in pcs if p[2] > 0]

    def sequence(g):
        seq = []
        for s in range(2 * g - (g == 0), 2 * g + 2):
            seq += cut(0, PH + 256 * s, A_S) + cut(1, PH + 256 * s, B_S)
        return seq

    def sem_slot(v, g, i):
        return hkv if (v and g == last and i < TRIG) else g

    def view(slot, v, t, lo, n):
        return kv_all.at[slot, v, pl.ds(1, rep), pl.ds(lo, n)] if t else kv_all.at[slot, v, 0, pl.ds(lo, n)]

    def start_packet(bu, g):
        slot = bu % 2
        for i, (t, lo, n) in enumerate(sequence(g)):
            for v in range(2):
                src = ((kb_hbm, vb_hbm)[v].at[pl.ds(bu * rep, rep), pl.ds(lo, n)] if t
                       else (ka_hbm, va_hbm)[v].at[bu, pl.ds(lo, n)])
                pltpu.make_async_copy(src, view(slot, v, t, lo, n),
                                      sems[v].at[slot, sem_slot(v, g, i)]).start(priority=v)

    par = b % 2

    def wait_all(ref, sem):
        pltpu.make_async_copy(ref, ref, sem).wait()

    def wait_kv(v, slot):
        g = min(slot, last)
        pcs = sorted(p for i, p in enumerate(sequence(g)) if sem_slot(v, g, i) == slot)
        runs = []
        for t, lo, n in pcs:
            if runs and runs[-1][0] == t and runs[-1][1] + runs[-1][2] == lo:
                runs[-1][2] += n
            else:
                runs.append([t, lo, n])
        for t, lo, n in runs:
            wait_all(view(par, v, t, lo, n), sems[v].at[par, slot])

    def b_heads(g):
        return [g + hkv * r for r in range(rep)]

    def q_proj(bu, g):
        r0 = pl.multiple_of(bu * sq, sq)
        w = (wq_buf[0, :, g * gw:(g + 1) * gw],
             jnp.concatenate([wq_buf[1, :, h * dh:(h + 1) * dh] for h in b_heads(g)], axis=1))
        for i in range(2):
            q = (jnp.dot(x_buf[i, pl.ds(r0, sq), :], w[i],
                         preferred_element_type=jnp.float32) * qscale).astype(jnp.bfloat16)
            for r in range(rep):
                q_buf[i, g, r * sq:(r + 1) * sq, :] = q[:, r * dh:(r + 1) * dh]

    @pl.when(b == 0)
    def _prologue():
        ns = 64
        rr = lambda t: (t % RR) * (ns // RR) + t // RR

        def copy2(srcs, dst, idx, sem, prio=lambda i: i):
            for i in range(2):
                pltpu.make_async_copy(srcs[i].at[idx], dst.at[(i,) + idx], sem(i)).start(priority=prio(i))

        def row_stripe(srcs, dst, s, n, sem):
            r0 = pl.multiple_of(s * 64, 64)
            r1 = pl.multiple_of(((s + 1) % n) * 64, 64)
            if WOX:
                copy2(srcs, dst, (pl.ds(r0 + 24, 8), pl.ds(128, 384)), sem)
                copy2(srcs, dst, (pl.ds(r0 + 32, 32),), sem)
                copy2(srcs, dst, (pl.ds(r1, 24),), sem)
                copy2(srcs, dst, (pl.ds(r1 + 24, 8), pl.ds(0, 128)), sem)
            else:
                copy2(srcs, dst, (pl.ds(r0 + 24, 40),), sem)
                copy2(srcs, dst, (pl.ds(r1, 24),), sem)

        def x_body(j, carry):
            copy2((xa_hbm, xb_hbm), x_buf, (pl.ds(pl.multiple_of(j * XP, 8), XP),), lambda i: w_sems.at[0], lambda i: 1)
            return carry

        def wq_body(t, carry):
            s = rr(t)
            if XM == 1:
                @pl.when(t % 8 == 0)
                def _():
                    row_stripe((xa_hbm, xb_hbm), x_buf, t // 8, 8, lambda i: w_sems.at[0])
            c = WQT * 128
            copy2((wqa_hbm, wqb_hbm), wq_buf, (pl.ds(pl.multiple_of(s * 8, 8), 8), pl.ds(c, 4096 - c)), lambda i: w_sems.at[1])
            copy2((wqa_hbm, wqb_hbm), wq_buf, (pl.ds(pl.multiple_of(((s + 1) % ns) * 8, 8), 8), pl.ds(0, c)), lambda i: w_sems.at[1])
            return carry

        def wo_body(t, carry):
            row_stripe((woa_hbm, wob_hbm), wo_buf, rr(t), ns, lambda i: w_sems.at[2])
            return carry

        if XM == 0:
            lax.fori_loop(0, nb * sq // XP, x_body, 0)
        lax.fori_loop(0, ns, wq_body, 0)
        lax.fori_loop(0, ns, wo_body, 0)
        start_packet(0, 0)
        wait_all(x_buf, w_sems.at[0])
        wait_all(wq_buf, w_sems.at[1])
        for g in range(hkv):
            if g % PACE == 0 and g // PACE + 1 < LA:
                start_packet(0, g // PACE + 1)
            if not NOCOMP:
                q_proj(0, g)
        wait_all(wo_buf, w_sems.at[2])

    def head(v, j, g):
        return kv_all[par, v, j, g * sk:(g + 1) * sk, :]

    def qk_unit(g):
        return ([_softmax_parts(q_buf[0, g], head(0, 0, g))]
                + [_softmax_parts(q_buf[1, g, r * sq:(r + 1) * sq, :], head(0, 1 + r, g))
                   for r in range(rep)])

    def pv_unit(g, res):
        o = _pv(*res[0], head(1, 0, g))
        oa = jnp.concatenate([o[r * sq:(r + 1) * sq, :] for r in range(rep)], axis=1)
        ob = jnp.concatenate([_pv(*res[1 + r], head(1, 1 + r, g)) for r in range(rep)], axis=1)
        return oa, ob

    def out_proj(g, o, y):
        w = (wo_buf[0, g * gw:(g + 1) * gw, :],
             jnp.concatenate([wo_buf[1, h * dh:(h + 1) * dh, :] for h in b_heads(g)], axis=0))
        z = [jnp.dot(o[i], w[i], preferred_element_type=jnp.float32) for i in range(2)]
        return z if y is None else [z[0] + y[0], z[1] + y[1]]

    def store_rows(r, n, priority):
        pltpu.make_async_copy(o_buf.at[pl.ds(r, n)], out_hbm.at[pl.ds(r, n)],
                              w_sems.at[0]).start(priority=priority)

    y = None
    wait_kv(0, 0)
    res = None if NOCOMP else qk_unit(0)
    for g in range(hkv):
        if g < last:
            wait_kv(0, g + 1)
        else:
            pl.when(b < NB - 1)(lambda: wait_kv(1, hkv))
        wait_kv(1, g)

        bu, gu = b + (g + LA) // hkv, (g + LA) % hkv
        pl.when(bu < NB)(lambda: start_packet(bu, gu))

        if not NOCOMP:
            pl.when(b < NB - 1)(lambda: q_proj(b + 1, g))
            o = pv_unit(g, res)
        if g == last - 1:
            @pl.when(b == NB - 1)
            def _():
                wait_kv(1, hkv)
                if WR:
                    store_rows(0, (nb - 1) * sq, 1)
        if NOCOMP:
            y = [jnp.zeros((sq, d), jnp.float32)] * 2
            continue
        if g < last:
            res = qk_unit(g + 1)
        y = out_proj(g, o, y)

    r0 = pl.multiple_of(b * sq, sq)
    o_buf[pl.ds(r0, sq), 0:d] = y[0].astype(o_buf.dtype)
    o_buf[pl.ds(r0, sq), d:2 * d] = y[1].astype(o_buf.dtype)

    @pl.when(b == NB - 1)
    def _():
        if WR:
            store_rows((nb - 1) * sq, sq, 0)
            pltpu.make_async_copy(o_buf, out_hbm, w_sems.at[0]).wait()


@jax.jit
def pallas_concat_heads__gqa_block_cached__mha_block_cached__near_ridge_kernel(
    A_x, A_k_cache, A_v_cache, A_wq, A_wo, B_x, B_k_cache, B_v_cache, B_wq, B_wo,
):
    B, Sq, D = A_x.shape
    _, Hkv, Sk, Dh = A_k_cache.shape
    H = B_k_cache.shape[1]
    rep = H // Hkv
    qscale = (Dh ** -0.5) * _LOG2E
    dt = A_x.dtype
    grp = lambda a: a.reshape(-1, Hkv * Sk, Dh)

    hbm = pl.BlockSpec(memory_space=pl.ANY)
    out = pl.pallas_call(
        functools.partial(_kernel, nb=B, sq=Sq, sk=Sk, dh=Dh, rep=rep, d=D, hkv=Hkv, qscale=qscale),
        grid=(NB,),
        in_specs=[hbm] * 10,
        out_specs=hbm,
        out_shape=jax.ShapeDtypeStruct((B * Sq, 2 * D), dt),
        scratch_shapes=[
            pltpu.VMEM((B * Sq, 2 * D), dt),
            pltpu.VMEM((2, B * Sq, D), dt),
            pltpu.VMEM((2, D, H * Dh), dt),
            pltpu.VMEM((2, H * Dh, D), dt),
            pltpu.VMEM((2, Hkv, rep * Sq, Dh), dt),
            pltpu.VMEM((2, 2, 1 + rep, Hkv * Sk, Dh), dt),
            pltpu.SemaphoreType.DMA((2, Hkv)),
            pltpu.SemaphoreType.DMA((2, Hkv + 1)),
            pltpu.SemaphoreType.DMA((3,)),
        ],
        compiler_params=pltpu.CompilerParams(
            dimension_semantics=("arbitrary",),
            vmem_limit_bytes=64 * 1024 * 1024,
            disable_bounds_checks=True,
            disable_semaphore_checks=True,
        ),
    )(A_x.reshape(B * Sq, D), grp(A_k_cache), grp(A_v_cache), A_wq, A_wo,
      B_x.reshape(B * Sq, D), grp(B_k_cache), grp(B_v_cache), B_wq, B_wo)
    return out.reshape(B, Sq, 2 * D)
```

```python
import functools
import math

import jax
import jax.numpy as jnp
from jax import lax
import jax.experimental.pallas as pl
import jax.experimental.pallas.tpu as pltpu

_NT = (((1,), (1,)), ((), ()))
_LOG2E = math.log2(math.e)

_STRIPE = 32
_PHASE = 13
_A_ROWS = 128
_B_ROWS = 32
_SPREAD = 4
_X_ROWS = 32
_LOOKAHEAD = 4
_TRIGGER = 8


def _softmax_parts(q, k):
    s = lax.dot_general(q, k, _NT, preferred_element_type=jnp.float32)
    m = jnp.max(s, axis=-1, keepdims=True)
    p = jnp.exp2(s - m)
    l = jnp.sum(p, axis=-1, keepdims=True)
    r = pl.reciprocal(l, approx=True)
    r = r * (2.0 - l * r)
    return p.astype(jnp.bfloat16), r


def _pv(p, r, v):
    o = jnp.dot(p, v, preferred_element_type=jnp.float32)
    return (o * r).astype(jnp.bfloat16)


def _kv_packets(rows, sk):
    stream = []
    for s0 in range(8 * (_PHASE - _STRIPE), rows, 8 * _STRIPE):
        for is_b, n in enumerate((_A_ROWS, _B_ROWS)):
            for lo in range(s0, s0 + 8 * _STRIPE, n):
                lo, hi = max(lo, 0), min(lo + n, rows)
                if lo < hi:
                    stream.append((is_b, lo, hi - lo))
    packets = [[] for _ in range(rows // sk)]
    for i, copy in enumerate(stream):
        packets[min(c[1] // sk for c in stream[i:])].append(copy)
    return packets


def _kernel(xa_hbm, ka_hbm, va_hbm, wqa_hbm, woa_hbm,
            xb_hbm, kb_hbm, vb_hbm, wqb_hbm, wob_hbm,
            out_hbm,
            o_buf, x_buf, wq_buf, wo_buf, q_buf, kv_buf, k_sems, v_sems, w_sems,
            *, nb, sq, sk, dh, rep, d, hkv, qscale):
    b = pl.program_id(0)
    gw = rep * dh
    last = hkv - 1
    packets = _kv_packets(hkv * sk, sk)
    kv_sems = (k_sems, v_sems)

    def sem_slot(v, g, i):
        return hkv if (v and g == last and i < _TRIGGER) else g

    def kv_view(slot, v, is_b, lo, n):
        return kv_buf.at[slot, v, pl.ds(is_b, rep if is_b else 1), pl.ds(lo, n)]

    def start_packet(bu, g):
        slot = bu % 2
        for i, (is_b, lo, n) in enumerate(packets[g]):
            for v in range(2):
                src = ((kb_hbm, vb_hbm)[v].at[pl.ds(bu * rep, rep), pl.ds(lo, n)] if is_b
                       else (ka_hbm, va_hbm)[v].at[pl.ds(bu, 1), pl.ds(lo, n)])
                pltpu.make_async_copy(src, kv_view(slot, v, is_b, lo, n),
                                      kv_sems[v].at[slot, sem_slot(v, g, i)]).start(priority=v)

    par = b % 2

    def wait_all(ref, sem):
        pltpu.make_async_copy(ref, ref, sem).wait()

    def wait_kv(v, slot):
        g = min(slot, last)
        mine = [c for i, c in enumerate(packets[g]) if sem_slot(v, g, i) == slot]
        for is_b in range(2):
            part = [c for c in mine if c[0] == is_b]
            wait_all(kv_view(par, v, is_b, part[0][1], sum(c[2] for c in part)),
                     kv_sems[v].at[par, slot])

    def b_heads(g):
        return [g + hkv * r for r in range(rep)]

    def q_proj(bu, g):
        r0 = pl.multiple_of(bu * sq, sq)
        w = (wq_buf[0, :, g * gw:(g + 1) * gw],
             jnp.concatenate([wq_buf[1, :, h * dh:(h + 1) * dh] for h in b_heads(g)], axis=1))
        for i in range(2):
            q = (jnp.dot(x_buf[i, pl.ds(r0, sq), :], w[i],
                         preferred_element_type=jnp.float32) * qscale).astype(jnp.bfloat16)
            for r in range(rep):
                q_buf[i, g, r * sq:(r + 1) * sq, :] = q[:, r * dh:(r + 1) * dh]

    @pl.when(b == 0)
    def _prologue():
        def copy_ab(srcs, dst, sem, r, n, c0=0, c1=None, priority=None):
            c1 = dst.shape[-1] if c1 is None else c1
            idx = (pl.ds(pl.multiple_of(r, 8), n), pl.ds(c0, c1 - c0))
            for i in range(2):
                pltpu.make_async_copy(srcs[i].at[idx], dst.at[(i,) + idx], w_sems.at[sem]).start(
                    priority=i if priority is None else priority)

        def x_body(j, carry):
            copy_ab((xa_hbm, xb_hbm), x_buf, 0, j * _X_ROWS, _X_ROWS, priority=1)
            return carry

        def weight_loop(srcs, dst, sem):
            tiles = dst.shape[-1] // 128
            per, ro, co = max(8 * _STRIPE // tiles, 8), _PHASE // tiles * 8, _PHASE % tiles * 128
            n = dst.shape[-2] // per

            def body(t, carry):
                s = (t % _SPREAD) * (n // _SPREAD) + t // _SPREAD
                r0, r1 = s * per, ((s + 1) % n) * per
                copy_ab(srcs, dst, sem, r0 + ro, 8, c0=co)
                if per > 8:
                    copy_ab(srcs, dst, sem, r0 + ro + 8, per - ro - 8)
                    copy_ab(srcs, dst, sem, r1, ro)
                copy_ab(srcs, dst, sem, r1 + ro, 8, c1=co)
                return carry

            lax.fori_loop(0, n, body, 0)

        lax.fori_loop(0, nb * sq // _X_ROWS, x_body, 0)
        weight_loop((wqa_hbm, wqb_hbm), wq_buf, 1)
        weight_loop((woa_hbm, wob_hbm), wo_buf, 2)
        start_packet(0, 0)
        wait_all(x_buf, w_sems.at[0])
        wait_all(wq_buf, w_sems.at[1])
        for g in range(hkv):
            if g % 2 == 0 and g // 2 + 1 < _LOOKAHEAD:
                start_packet(0, g // 2 + 1)
            q_proj(0, g)
        wait_all(wo_buf, w_sems.at[2])

    def head(v, j, g):
        return kv_buf[par, v, j, g * sk:(g + 1) * sk, :]

    def qk_unit(g):
        return ([_softmax_parts(q_buf[0, g], head(0, 0, g))]
                + [_softmax_parts(q_buf[1, g, r * sq:(r + 1) * sq, :], head(0, 1 + r, g))
                   for r in range(rep)])

    def pv_unit(g, res):
        o = _pv(*res[0], head(1, 0, g))
        oa = jnp.concatenate([o[r * sq:(r + 1) * sq, :] for r in range(rep)], axis=1)
        ob = jnp.concatenate([_pv(*res[1 + r], head(1, 1 + r, g)) for r in range(rep)], axis=1)
        return oa, ob

    def out_proj(g, o, y):
        w = (wo_buf[0, g * gw:(g + 1) * gw, :],
             jnp.concatenate([wo_buf[1, h * dh:(h + 1) * dh, :] for h in b_heads(g)], axis=0))
        z = [jnp.dot(o[i], w[i], preferred_element_type=jnp.float32) for i in range(2)]
        return z if y is None else [z[0] + y[0], z[1] + y[1]]

    def store_rows(r, n, priority):
        pltpu.make_async_copy(o_buf.at[pl.ds(r, n)], out_hbm.at[pl.ds(r, n)],
                              w_sems.at[0]).start(priority=priority)

    y = None
    wait_kv(0, 0)
    res = qk_unit(0)
    for g in range(hkv):
        if g < last:
            wait_kv(0, g + 1)
        else:
            pl.when(b < nb - 1)(lambda: wait_kv(1, hkv))
        wait_kv(1, g)

        bu, gu = b + (g + _LOOKAHEAD) // hkv, (g + _LOOKAHEAD) % hkv
        pl.when(bu < nb)(lambda: start_packet(bu, gu))
        pl.when(b < nb - 1)(lambda: q_proj(b + 1, g))

        o = pv_unit(g, res)
        if g == last - 1:
            @pl.when(b == nb - 1)
            def _():
                wait_kv(1, hkv)
                store_rows(0, (nb - 1) * sq, 1)
        if g < last:
            res = qk_unit(g + 1)
        y = out_proj(g, o, y)

    r0 = pl.multiple_of(b * sq, sq)
    o_buf[pl.ds(r0, sq), 0:d] = y[0].astype(o_buf.dtype)
    o_buf[pl.ds(r0, sq), d:2 * d] = y[1].astype(o_buf.dtype)

    @pl.when(b == nb - 1)
    def _():
        store_rows((nb - 1) * sq, sq, 0)
        pltpu.make_async_copy(o_buf, out_hbm, w_sems.at[0]).wait()


@jax.jit
def pallas_concat_heads__gqa_block_cached__mha_block_cached__near_ridge_kernel(
    A_x, A_k_cache, A_v_cache, A_wq, A_wo, B_x, B_k_cache, B_v_cache, B_wq, B_wo,
):
    B, Sq, D = A_x.shape
    _, Hkv, Sk, Dh = A_k_cache.shape
    H = B_k_cache.shape[1]
    rep = H // Hkv
    qscale = (Dh ** -0.5) * _LOG2E
    dt = A_x.dtype
    groups = lambda a: a.reshape(-1, Hkv * Sk, Dh)

    hbm = pl.BlockSpec(memory_space=pl.ANY)
    out = pl.pallas_call(
        functools.partial(_kernel, nb=B, sq=Sq, sk=Sk, dh=Dh, rep=rep, d=D, hkv=Hkv, qscale=qscale),
        grid=(B,),
        in_specs=[hbm] * 10,
        out_specs=hbm,
        out_shape=jax.ShapeDtypeStruct((B * Sq, 2 * D), dt),
        scratch_shapes=[
            pltpu.VMEM((B * Sq, 2 * D), dt),
            pltpu.VMEM((2, B * Sq, D), dt),
            pltpu.VMEM((2, D, H * Dh), dt),
            pltpu.VMEM((2, H * Dh, D), dt),
            pltpu.VMEM((2, Hkv, rep * Sq, Dh), dt),
            pltpu.VMEM((2, 2, 1 + rep, Hkv * Sk, Dh), dt),
            pltpu.SemaphoreType.DMA((2, Hkv)),
            pltpu.SemaphoreType.DMA((2, Hkv + 1)),
            pltpu.SemaphoreType.DMA((3,)),
        ],
        compiler_params=pltpu.CompilerParams(
            dimension_semantics=("arbitrary",),
            vmem_limit_bytes=64 * 1024 * 1024,
            disable_bounds_checks=True,
            disable_semaphore_checks=True,
        ),
    )(A_x.reshape(B * Sq, D), groups(A_k_cache), groups(A_v_cache), A_wq, A_wo,
      B_x.reshape(B * Sq, D), groups(B_k_cache), groups(B_v_cache), B_wq, B_wo)
    return out.reshape(B, Sq, 2 * D)
```

```python
import functools
import math

import jax
import jax.numpy as jnp
from jax import lax
import jax.experimental.pallas as pl
import jax.experimental.pallas.tpu as pltpu

_NT = (((1,), (1,)), ((), ()))
_LOG2E = math.log2(math.e)

_STRIPE = 32
_PHASE = 13
_A_ROWS = 128
_B_ROWS = 32
_SPREAD = 4
_X_ROWS = 32
_LOOKAHEAD = 4
_TRIGGER = 9


def _softmax_parts(q, k):
    s = lax.dot_general(q, k, _NT, preferred_element_type=jnp.float32)
    m = jnp.max(s, axis=-1, keepdims=True)
    p = jnp.exp2(s - m)
    l = jnp.sum(p, axis=-1, keepdims=True)
    r = pl.reciprocal(l, approx=True)
    r = r * (2.0 - l * r)
    return p.astype(jnp.bfloat16), r


def _pv(p, r, v):
    o = jnp.dot(p, v, preferred_element_type=jnp.float32)
    return (o * r).astype(jnp.bfloat16)


def _kv_packets(rows, sk):
    stream = []
    for s0 in range(8 * (_PHASE - _STRIPE), rows, 8 * _STRIPE):
        for is_b, n in enumerate((_A_ROWS, _B_ROWS)):
            for lo in range(s0, s0 + 8 * _STRIPE, n):
                lo, hi = max(lo, 0), min(lo + n, rows)
                if lo < hi:
                    stream.append((is_b, lo, hi - lo))
    packets = [[] for _ in range(rows // sk)]
    for i, copy in enumerate(stream):
        packets[min(c[1] // sk for c in stream[i:])].append(copy)
    return packets


def _kernel(xa_hbm, ka_hbm, va_hbm, wqa_hbm, woa_hbm,
            xb_hbm, kb_hbm, vb_hbm, wqb_hbm, wob_hbm,
            out_hbm,
            o_buf, x_buf, wq_buf, wo_buf, q_buf, kv_buf, k_sems, v_sems, w_sems,
            *, nb, sq, sk, dh, rep, d, hkv, qscale):
    b = pl.program_id(0)
    gw = rep * dh
    last = hkv - 1
    packets = _kv_packets(hkv * sk, sk)
    kv_sems = (k_sems, v_sems)

    def sem_slot(v, g, i):
        return hkv if (v and g == last and i < _TRIGGER) else g

    def kv_view(slot, v, is_b, lo, n):
        return kv_buf.at[slot, v, pl.ds(is_b, rep if is_b else 1), pl.ds(lo, n)]

    def start_packet(bu, g):
        slot = bu % 2
        for i, (is_b, lo, n) in enumerate(packets[g]):
            for v in range(2):
                src = ((kb_hbm, vb_hbm)[v].at[pl.ds(bu * rep, rep), pl.ds(lo, n)] if is_b
                       else (ka_hbm, va_hbm)[v].at[pl.ds(bu, 1), pl.ds(lo, n)])
                pltpu.make_async_copy(src, kv_view(slot, v, is_b, lo, n),
                                      kv_sems[v].at[slot, sem_slot(v, g, i)]).start(priority=v)

    par = b % 2

    def wait_all(ref, sem):
        pltpu.make_async_copy(ref, ref, sem).wait()

    def wait_kv(v, slot):
        g = min(slot, last)
        mine = [c for i, c in enumerate(packets[g]) if sem_slot(v, g, i) == slot]
        for is_b in range(2):
            part = [c for c in mine if c[0] == is_b]
            wait_all(kv_view(par, v, is_b, part[0][1], sum(c[2] for c in part)),
                     kv_sems[v].at[par, slot])

    def b_heads(g):
        return [g + hkv * r for r in range(rep)]

    def q_proj(bu, g):
        r0 = pl.multiple_of(bu * sq, sq)
        w = (wq_buf[0, :, g * gw:(g + 1) * gw],
             jnp.concatenate([wq_buf[1, :, h * dh:(h + 1) * dh] for h in b_heads(g)], axis=1))
        for i in range(2):
            q = (jnp.dot(x_buf[i, pl.ds(r0, sq), :], w[i],
                         preferred_element_type=jnp.float32) * qscale).astype(jnp.bfloat16)
            for r in range(rep):
                q_buf[i, g, r * sq:(r + 1) * sq, :] = q[:, r * dh:(r + 1) * dh]

    @pl.when(b == 0)
    def _prologue():
        def copy_ab(srcs, dst, sem, r, n, c0=0, c1=None, priority=None):
            c1 = dst.shape[-1] if c1 is None else c1
            idx = (pl.ds(pl.multiple_of(r, 8), n), pl.ds(c0, c1 - c0))
            for i in range(2):
                pltpu.make_async_copy(srcs[i].at[idx], dst.at[(i,) + idx], w_sems.at[sem]).start(
                    priority=i if priority is None else priority)

        def x_body(j, carry):
            copy_ab((xa_hbm, xb_hbm), x_buf, 0, j * _X_ROWS, _X_ROWS, priority=1)
            return carry

        def weight_loop(srcs, dst, sem):
            tiles = dst.shape[-1] // 128
            per, ro, co = max(8 * _STRIPE // tiles, 8), _PHASE // tiles * 8, _PHASE % tiles * 128
            n = dst.shape[-2] // per

            def body(t, carry):
                s = (t % _SPREAD) * (n // _SPREAD) + t // _SPREAD
                r0, r1 = s * per, ((s + 1) % n) * per
                copy_ab(srcs, dst, sem, r0 + ro, 8, c0=co)
                if per > 8:
                    copy_ab(srcs, dst, sem, r0 + ro + 8, per - ro - 8)
                    copy_ab(srcs, dst, sem, r1, ro)
                copy_ab(srcs, dst, sem, r1 + ro, 8, c1=co)
                return carry

            lax.fori_loop(0, n, body, 0)

        lax.fori_loop(0, nb * sq // _X_ROWS, x_body, 0)
        weight_loop((wqa_hbm, wqb_hbm), wq_buf, 1)
        weight_loop((woa_hbm, wob_hbm), wo_buf, 2)
        start_packet(0, 0)
        wait_all(x_buf, w_sems.at[0])
        wait_all(wq_buf, w_sems.at[1])
        for g in range(hkv):
            if g % 2 == 0 and g // 2 + 1 < _LOOKAHEAD:
                start_packet(0, g // 2 + 1)
            q_proj(0, g)
        wait_all(wo_buf, w_sems.at[2])

    def head(v, j, g):
        return kv_buf[par, v, j, g * sk:(g + 1) * sk, :]

    def qk_unit(g):
        return ([_softmax_parts(q_buf[0, g], head(0, 0, g))]
                + [_softmax_parts(q_buf[1, g, r * sq:(r + 1) * sq, :], head(0, 1 + r, g))
                   for r in range(rep)])

    def pv_unit(g, res):
        o = _pv(*res[0], head(1, 0, g))
        oa = jnp.concatenate([o[r * sq:(r + 1) * sq, :] for r in range(rep)], axis=1)
        ob = jnp.concatenate([_pv(*res[1 + r], head(1, 1 + r, g)) for r in range(rep)], axis=1)
        return oa, ob

    def out_proj(g, o, y):
        w = (wo_buf[0, g * gw:(g + 1) * gw, :],
             jnp.concatenate([wo_buf[1, h * dh:(h + 1) * dh, :] for h in b_heads(g)], axis=0))
        z = [jnp.dot(o[i], w[i], preferred_element_type=jnp.float32) for i in range(2)]
        return z if y is None else [z[0] + y[0], z[1] + y[1]]

    def store_rows(r, n, priority):
        pltpu.make_async_copy(o_buf.at[pl.ds(r, n)], out_hbm.at[pl.ds(r, n)],
                              w_sems.at[0]).start(priority=priority)

    y = None
    wait_kv(0, 0)
    res = qk_unit(0)
    for g in range(hkv):
        if g < last:
            wait_kv(0, g + 1)
        else:
            pl.when(b < nb - 1)(lambda: wait_kv(1, hkv))
        wait_kv(1, g)

        bu, gu = b + (g + _LOOKAHEAD) // hkv, (g + _LOOKAHEAD) % hkv
        pl.when(bu < nb)(lambda: start_packet(bu, gu))
        pl.when(b < nb - 1)(lambda: q_proj(b + 1, g))

        o = pv_unit(g, res)
        if g == last - 1:
            @pl.when(b == nb - 1)
            def _():
                wait_kv(1, hkv)
                for j in sorted(range(nb - 1), key=lambda j: j % (nb // 2)):
                    for r in range(j * sq, (j + 1) * sq, sq // 2):
                        store_rows(r, sq // 2, 1)
        if g < last:
            res = qk_unit(g + 1)
        y = out_proj(g, o, y)

    r0 = pl.multiple_of(b * sq, sq)
    o_buf[pl.ds(r0, sq), 0:d] = y[0].astype(o_buf.dtype)
    o_buf[pl.ds(r0, sq), d:2 * d] = y[1].astype(o_buf.dtype)

    @pl.when(b == nb - 1)
    def _():
        store_rows((nb - 1) * sq, sq, 0)
        pltpu.make_async_copy(o_buf, out_hbm, w_sems.at[0]).wait()


@jax.jit
def pallas_concat_heads__gqa_block_cached__mha_block_cached__near_ridge_kernel(
    A_x, A_k_cache, A_v_cache, A_wq, A_wo, B_x, B_k_cache, B_v_cache, B_wq, B_wo,
):
    B, Sq, D = A_x.shape
    _, Hkv, Sk, Dh = A_k_cache.shape
    H = B_k_cache.shape[1]
    rep = H // Hkv
    qscale = (Dh ** -0.5) * _LOG2E
    dt = A_x.dtype
    groups = lambda a: a.reshape(-1, Hkv * Sk, Dh)

    hbm = pl.BlockSpec(memory_space=pl.ANY)
    out = pl.pallas_call(
        functools.partial(_kernel, nb=B, sq=Sq, sk=Sk, dh=Dh, rep=rep, d=D, hkv=Hkv, qscale=qscale),
        grid=(B,),
        in_specs=[hbm] * 10,
        out_specs=hbm,
        out_shape=jax.ShapeDtypeStruct((B * Sq, 2 * D), dt),
        scratch_shapes=[
            pltpu.VMEM((B * Sq, 2 * D), dt),
            pltpu.VMEM((2, B * Sq, D), dt),
            pltpu.VMEM((2, D, H * Dh), dt),
            pltpu.VMEM((2, H * Dh, D), dt),
            pltpu.VMEM((2, Hkv, rep * Sq, Dh), dt),
            pltpu.VMEM((2, 2, 1 + rep, Hkv * Sk, Dh), dt),
            pltpu.SemaphoreType.DMA((2, Hkv)),
            pltpu.SemaphoreType.DMA((2, Hkv + 1)),
            pltpu.SemaphoreType.DMA((3,)),
        ],
        compiler_params=pltpu.CompilerParams(
            dimension_semantics=("arbitrary",),
            vmem_limit_bytes=64 * 1024 * 1024,
            disable_bounds_checks=True,
            disable_semaphore_checks=True,
        ),
    )(A_x.reshape(B * Sq, D), groups(A_k_cache), groups(A_v_cache), A_wq, A_wo,
      B_x.reshape(B * Sq, D), groups(B_k_cache), groups(B_v_cache), B_wq, B_wo)
    return out.reshape(B, Sq, 2 * D)
```
